```python
import jax
import jax.numpy as jnp

def _softmax(x, axis=-1):
    return jax.nn.softmax(x, axis=axis)
def _gelu(x):
    return jax.nn.gelu(x, approximate=True)
def _silu(x):
    return jax.nn.silu(x)
def _sigmoid(x):
    return jax.nn.sigmoid(x)
def _layernorm(x, axis=-1, eps=1e-5):
    m = jnp.mean(x, axis=axis, keepdims=True)
    v = jnp.var(x, axis=axis, keepdims=True)
    return (x - m) / jnp.sqrt(v + eps)
def _scatter_add(tgt, idx, src, axis=0):
    return tgt.at[idx].add(src)
def _segment_sum(src, seg, n):
    return jax.ops.segment_sum(src, seg, n)
class _Rng:
    def __init__(self, key):
        self._k = key
    def _next(self):
        self._k, sub = jax.random.split(self._k)
        return sub
    def normal(self, shape):
        return jax.random.normal(self._next(), shape, dtype=jnp.bfloat16)
    def randint(self, lo, hi, shape):
        return jax.random.randint(self._next(), shape, lo, hi, dtype=jnp.int32)
    def uniform(self, shape, lo=0.0, hi=1.0):
        return jax.random.uniform(self._next(), shape, jnp.bfloat16, lo, hi)
    def permutation(self, n):
        return jax.random.permutation(self._next(), n)


kernel_name = 'gated_mix__mha_block_cached__compressed_kv_cla__decode'

def setup_inputs():
    _rng = _Rng(jax.random.key(int.from_bytes(__import__("os").urandom(4), "little")))
    _w = (lambda a: (lambda t: t.astype(jnp.bfloat16) if jnp.issubdtype(t.dtype, jnp.floating) else t)(jnp.asarray(a)))
    def _A_setup():
        B, Sq, D = 2, 1, 512
        H, Sk, Dh = 32, 8192, 128
        return {
            "x": _w((lambda *s: _rng.normal(s) * 0.05)(B, Sq, D)),
            "k_cache": _w((lambda *s: _rng.normal(s) * 0.05)(B, H, Sk, Dh)),
            "v_cache": _w((lambda *s: _rng.normal(s) * 0.05)(B, H, Sk, Dh)),
            "wq": _w((lambda *s: _rng.normal(s) * 0.05)(D, H * Dh) * (D ** -0.5)),
            "wo": _w((lambda *s: _rng.normal(s) * 0.05)(H * Dh, D) * ((H * Dh) ** -0.5)),
        }
    _A_in = _A_setup()

    def _B_setup():
        B, H, Sq, Sk, D, M = 2, 32, 1, 8192, 128, 512
        Dc = 4 * D
        return {
            "x": _w((lambda *s: _rng.normal(s) * 0.05)(B, Sq, M)),
            "c_kv": _w((lambda *s: _rng.normal(s) * 0.05)(B, Sk, Dc)),
            "w_q": _w((lambda *s: _rng.normal(s) * 0.05)(M, H, D) * (M ** -0.5)),
            "w_uk": _w((lambda *s: _rng.normal(s) * 0.05)(Dc, H, D) * (Dc ** -0.5)),
            "w_uv": _w((lambda *s: _rng.normal(s) * 0.05)(Dc, H, D) * (Dc ** -0.5)),
            "w_o": _w((lambda *s: _rng.normal(s) * 0.05)(H, D, M) * ((H * D) ** -0.5)),
        }
    _B_in = _B_setup()

    return {
        "A_x": _A_in["x"],
        "A_k_cache": _A_in["k_cache"],
        "A_v_cache": _A_in["v_cache"],
        "A_wq": _A_in["wq"],
        "A_wo": _A_in["wo"],
        "B_x": _B_in["x"],
        "B_c_kv": _B_in["c_kv"],
        "B_w_q": _B_in["w_q"],
        "B_w_uk": _B_in["w_uk"],
        "B_w_uv": _B_in["w_uv"],
        "B_w_o": _B_in["w_o"],
        "gate_w": _w((lambda *s: _rng.normal(s) * 0.05)(512)),
    }

def reference(A_x, A_k_cache, A_v_cache, A_wq, A_wo, B_x, B_c_kv, B_w_q, B_w_uk, B_w_uv, B_w_o, gate_w):
    def _A_ref(x, k_cache, v_cache, wq, wo):
        B, Sq, D = x.shape
        H, Dh = 32, 128
        q = (lambda x, *d: x.transpose(*d))((x @ wq).reshape(B, Sq, H, Dh), 0, 2, 1, 3)
        scores = jnp.einsum("bhqd,bhkd->bhqk", q, k_cache) * (Dh ** -0.5)
        p = _softmax(scores, axis=-1)
        o = jnp.einsum("bhqk,bhkd->bhqd", p, v_cache)
        return (lambda x, *d: x.transpose(*d))(o, 0, 2, 1, 3).reshape(B, Sq, H * Dh) @ wo

    def _B_ref(x, c_kv, w_q, w_uk, w_uv, w_o):
        B, Sq, M = x.shape[0], x.shape[1], x.shape[2]
        Sk = c_kv.shape[1]
        H, D = w_q.shape[1], w_q.shape[2]
        q = jnp.einsum("bqm,mhd->bhqd", x, w_q)
        k = jnp.einsum("bkc,chd->bhkd", c_kv, w_uk)
        v = jnp.einsum("bkc,chd->bhkd", c_kv, w_uv)
        scores = jnp.einsum("bhqd,bhkd->bhqk", q, k) * (D ** -0.5)
        off = Sk - Sq
        qi = jnp.arange(Sq)[:, None]
        kj = jnp.arange(Sk)[None, :]
        cmask = kj <= (qi + off)
        scores = jnp.where(cmask[None, None], scores, -1e9)
        p = _softmax(scores, axis=-1)
        ctx = jnp.einsum("bhqk,bhkd->bhqd", p, v)
        return jnp.einsum("bhqd,hdm->bqm", ctx, w_o)

    x = A_x
    g = _sigmoid((x * gate_w).sum(-1, keepdims=True))
    a = _A_ref(x, A_k_cache, A_v_cache, A_wq, A_wo)
    b = _B_ref(x, B_c_kv, B_w_q, B_w_uk, B_w_uv, B_w_o)
    return g * a + (1 - g) * b
```

```python
import functools

import jax
import jax.numpy as jnp
from jax.experimental import pallas as pl
from jax.experimental.pallas import tpu as pltpu

B, H, SK, DH, DM, DC = 2, 32, 8192, 128, 512, 512
NSTEP = B * H
CK = 512
NCH = B * SK // CK
SCALE = DH ** -0.5
NT = (((1,), (1,)), ((), ()))
NN = (((1,), (0,)), ((), ()))
f32 = jnp.float32
bf16 = jnp.bfloat16


def _head_pair(w_u32, j4, r):
    nwin = (DM - 1) * (H // 2) + 4
    view = w_u32.at[pl.ds(pl.multiple_of(j4 * 4, 4), nwin), :]
    w = view[pl.ds(r, DM, stride=H // 2), :]
    lo = pltpu.bitcast(w << 16, f32).astype(bf16)
    hi = pltpu.bitcast(w & jnp.uint32(0xFFFF0000), f32).astype(bf16)
    return lo, hi


def _kernel(x_hbm, gw_hbm, k_hbm, v_hbm, wq_hbm, wo_hbm, ckv_hbm, bwq_hbm, wuk_hbm,
            wuv_hbm, bwo_hbm, out_ref,
            kbuf, vbuf, wq_v, wo_v, ckv_v, bwq_v, wuk_v, wuv_v, bwo_v,
            x_v, gw_v, xs, qs, qabs, macc, lacc, cacc, acca,
            ksem, vsem, csem, wsem, *, nbuf, nvc, early_k):
    VR = SK // nvc

    def kcopy(i, s):
        return pltpu.make_async_copy(k_hbm.at[i], kbuf.at[s], ksem.at[s])

    def vcopy(i, s, c):
        return pltpu.make_async_copy(v_hbm.at[i, pl.ds(c * VR, VR)], vbuf.at[s, pl.ds(c * VR, VR)],
                                     vsem.at[s * nvc + c])

    def vstart(i, s):
        for c in range(nvc):
            vcopy(i, s, c).start()

    def ccopy(c):
        return pltpu.make_async_copy(ckv_hbm.at[pl.ds(c * CK, CK)], ckv_v.at[c], csem.at[c])

    wq_c = pltpu.make_async_copy(wq_hbm, wq_v, wsem.at[0])
    wo_c = pltpu.make_async_copy(wo_hbm, wo_v, wsem.at[1])
    bwq_c = pltpu.make_async_copy(bwq_hbm, bwq_v, wsem.at[2])
    wuk_c = pltpu.make_async_copy(wuk_hbm, wuk_v, wsem.at[3])
    wuv_c = pltpu.make_async_copy(wuv_hbm, wuv_v, wsem.at[4])
    bwo_c = pltpu.make_async_copy(bwo_hbm, bwo_v, wsem.at[5])

    x_c = pltpu.make_async_copy(x_hbm, x_v, wsem.at[6])
    gw_c = pltpu.make_async_copy(gw_hbm, gw_v, wsem.at[7])

    x_c.start()
    gw_c.start()
    wq_c.start()
    wo_c.start()
    kcopy(0, 0).start()
    vstart(0, 0)
    bwq_c.start()
    wuk_c.start()
    for i in range(1, nbuf):
        kcopy(i, i).start()
        vstart(i, i)

    row8 = jax.lax.broadcasted_iota(jnp.int32, (8, DH), 0)

    xs[...] = jnp.zeros_like(xs)
    x_c.wait()
    gw_c.wait()
    xs[0:B, :] = x_v[...].astype(f32)
    xb = xs[...].astype(bf16)
    acca[...] = jnp.zeros_like(acca)

    wq_c.wait()
    for n in range(4):
        qn = jnp.dot(xb, wq_v[:, n * 1024:(n + 1) * 1024], preferred_element_type=f32)
        for t in range(8):
            qs[n * 8 + t] = qn[:, t * DH:(t + 1) * DH]
    wo_c.wait()

    def a_step(i):
        s_ = i % nbuf
        b = i // H
        h = i % H
        q = qs[h].astype(bf16)
        kcopy(i, s_).wait()
        s = jax.lax.dot_general(q, kbuf[s_], NT, preferred_element_type=f32)
        if early_k:
            @pl.when(i + nbuf < NSTEP)
            def _():
                kcopy(i + nbuf, s_).start()
        s = s * SCALE
        m = jnp.max(s, axis=1, keepdims=True)
        p = jnp.exp(s - m)
        l = jnp.sum(p, axis=1, keepdims=True)
        pb = p.astype(bf16)
        o = jnp.zeros((8, DH), f32)
        for c in range(nvc):
            vcopy(i, s_, c).wait()
            o = o + jnp.dot(pb[:, c * VR:(c + 1) * VR], vbuf[s_, c * VR:(c + 1) * VR, :],
                            preferred_element_type=f32)

        @pl.when(i + nbuf < NSTEP)
        def _():
            if not early_k:
                kcopy(i + nbuf, s_).start()
            vstart(i + nbuf, s_)

        o = jnp.where(row8 == b, o / l, 0.0).astype(bf16)
        w = wo_v[pl.ds(pl.multiple_of(h * DH, DH), DH), :]
        acca[...] += jnp.dot(o, w, preferred_element_type=f32)

    def b_chunk(c):
        b = c // (SK // CK)
        ccopy(c).wait()
        cc = ckv_v[c]
        qa = qabs[pl.ds(pl.multiple_of(b * H, H), H), :].astype(bf16)
        s = jax.lax.dot_general(qa, cc, NT, preferred_element_type=f32) * SCALE
        m_old = macc[b]
        m_new = jnp.maximum(m_old, jnp.max(s, axis=1, keepdims=True))
        alpha = jnp.exp(m_old - m_new)
        p = jnp.exp(s - m_new[:, 0:1])
        lacc[b] = alpha * lacc[b] + jnp.sum(p, axis=1, keepdims=True)
        macc[b] = m_new
        pv = jnp.dot(p.astype(bf16), cc, preferred_element_type=f32)
        cacc[b] = alpha[:, 0:1] * cacc[b] + pv

    a_step(jnp.int32(0))

    for c in range(NCH):
        ccopy(c).start()
    wuv_c.start()
    bwo_c.start()

    bwq_c.wait()
    wuk_c.wait()
    bwq_u = bwq_v.bitcast(jnp.uint32)
    wuk_u = wuk_v.bitcast(jnp.uint32)

    def bprol(j4, carry):
        for jr in range(4):
            wq0, wq1 = _head_pair(bwq_u, j4, jr)
            wk0, wk1 = _head_pair(wuk_u, j4, jr)
            for t, (wqh, wkh) in enumerate(((wq0, wk0), (wq1, wk1))):
                qh = jnp.dot(xb, wqh, preferred_element_type=f32).astype(bf16)
                r = jax.lax.dot_general(qh, wkh, NT, preferred_element_type=f32)
                for b in range(B):
                    qabs[pl.ds(b * H + j4 * 8 + 2 * jr + t, 1), :] = r[b:b + 1, :]
        return carry

    jax.lax.fori_loop(0, H // 8, bprol, 0)
    macc[...] = jnp.full(macc.shape, -jnp.inf, f32)
    lacc[...] = jnp.zeros_like(lacc)
    cacc[...] = jnp.zeros_like(cacc)

    def seg1(i, carry):
        a_step(i)
        b_chunk(i - 1)
        return carry

    jax.lax.fori_loop(1, NCH + 1, seg1, 0)

    wuv_c.wait()
    bwo_c.wait()
    wuv_u = wuv_v.bitcast(jnp.uint32)
    row16 = jax.lax.broadcasted_iota(jnp.int32, (16, DH), 0)

    for b in range(B):
        cacc[b] = cacc[b] / lacc[b][:, 0:1]

    def bepi(g, acc):
        lhs = jnp.concatenate(
            [cacc[b, pl.ds(pl.multiple_of(g * 8, 8), 8), :] for b in range(B)], axis=0).astype(bf16)
        for jr in range(4):
            wv0, wv1 = _head_pair(wuv_u, g, jr)
            for t, wv in enumerate((wv0, wv1)):
                hr = 2 * jr + t
                ctx = jnp.dot(lhs, wv, preferred_element_type=f32)
                ctx = jnp.where((row16 % 8) == hr, ctx, 0.0).astype(bf16)
                wo_h = bwo_v[pl.ds(pl.multiple_of((g * 8 + hr) * DH, DH), DH), :]
                acc = acc + jnp.dot(ctx, wo_h, preferred_element_type=f32)
        return acc

    accb = jax.lax.fori_loop(0, H // 8, bepi, jnp.zeros((16, DM), f32))
    outb = jnp.concatenate([jnp.sum(accb[b * 8:(b + 1) * 8], axis=0, keepdims=True) for b in range(B)], axis=0)

    xf = x_v[...].astype(f32)
    z = jnp.sum(xf * gw_v[...].astype(f32).reshape(1, DM), axis=1, keepdims=True)
    g = 1.0 / (1.0 + jnp.exp(-z))
    base = (1.0 - g) * outb

    def seg2(i, carry):
        a_step(i)
        return carry

    jax.lax.fori_loop(NCH + 1, NSTEP, seg2, 0)

    out = g * acca[0:B, :] + base
    out_ref[...] = out.astype(out_ref.dtype)


NBUF, NVC = 2, 4


@jax.jit
def pallas_gated_mix__mha_block_cached__compressed_kv_cla__decode_kernel(
    A_x, A_k_cache, A_v_cache, A_wq, A_wo, B_x, B_c_kv, B_w_q, B_w_uk, B_w_uv, B_w_o, gate_w,
):
    del B_x
    nbuf, nvc = NBUF, NVC
    any_spec = pl.BlockSpec(memory_space=pl.ANY)
    vmem_spec = pl.BlockSpec(memory_space=pltpu.VMEM)
    out = pl.pallas_call(
        functools.partial(_kernel, nbuf=nbuf, nvc=nvc, early_k=True),
        out_shape=jax.ShapeDtypeStruct((B, DM), bf16),
        in_specs=[any_spec] * 11,
        out_specs=vmem_spec,
        scratch_shapes=[
            pltpu.VMEM((nbuf, SK, DH), bf16),
            pltpu.VMEM((nbuf, SK, DH), bf16),
            pltpu.VMEM((DM, H * DH), bf16),
            pltpu.VMEM((H * DH, DM), bf16),
            pltpu.VMEM((NCH, CK, DC), bf16),
            pltpu.VMEM((DM * H, DH), bf16),
            pltpu.VMEM((DC * H, DH), bf16),
            pltpu.VMEM((DC * H, DH), bf16),
            pltpu.VMEM((H * DH, DM), bf16),
            pltpu.VMEM((B, DM), bf16),
            pltpu.VMEM((DM,), bf16),
            pltpu.VMEM((8, DM), f32),
            pltpu.VMEM((H, 8, DH), f32),
            pltpu.VMEM((B * H, DC), f32),
            pltpu.VMEM((B, H, 128), f32),
            pltpu.VMEM((B, H, 128), f32),
            pltpu.VMEM((B, H, DC), f32),
            pltpu.VMEM((8, DM), f32),
            pltpu.SemaphoreType.DMA((nbuf,)),
            pltpu.SemaphoreType.DMA((nbuf * nvc,)),
            pltpu.SemaphoreType.DMA((NCH,)),
            pltpu.SemaphoreType.DMA((8,)),
        ],
        compiler_params=pltpu.CompilerParams(vmem_limit_bytes=110 * 2**20),
    )(
        A_x.reshape(B, DM), gate_w,
        A_k_cache.reshape(NSTEP, SK, DH), A_v_cache.reshape(NSTEP, SK, DH),
        A_wq, A_wo, B_c_kv.reshape(B * SK, DC),
        B_w_q.reshape(DM * H, DH), B_w_uk.reshape(DC * H, DH), B_w_uv.reshape(DC * H, DH),
        B_w_o.reshape(H * DH, DM),
    )
    return out.reshape(B, 1, DM)
```

```python
import jax
import jax.numpy as jnp
from jax.experimental import pallas as pl
from jax.experimental.pallas import tpu as pltpu

B, H, SK, DH, DM, DC = 2, 32, 8192, 128, 512, 512
NSTEP = B * H
CP = 2048
NCP = B * SK // CP
CK = 512
VSZ = (3072, 3072, 2048)
VOFF = (0, 3072, 6144)
WOH = (H - 1) * DH
SCALE = DH ** -0.5
NT = (((1,), (1,)), ((), ()))
f32 = jnp.float32
bf16 = jnp.bfloat16

S_BPROL = 2
S_CKV = 5
S_BEPI = S_CKV + NCP
S_BASE = S_BEPI + 4


def _head_pair(w_u32, g, r):
    nwin = (DM - 1) * (H // 2) + 4
    view = w_u32.at[pl.ds(pl.multiple_of(g * 4, 4), nwin), :]
    w = view[pl.ds(r, DM, stride=H // 2), :]
    lo = pltpu.bitcast(w << 16, f32).astype(bf16)
    hi = pltpu.bitcast(w & jnp.uint32(0xFFFF0000), f32).astype(bf16)
    return lo, hi


def _kernel(x_hbm, gw_hbm, k_hbm, v_hbm, wq_hbm, wo_hbm, ckv_hbm, bwq_hbm, wuk_hbm,
            wuv_hbm, bwo_hbm, out_ref,
            kbuf, vbuf, wq_v, wo_v, ckv_v, bwq_v, wuk_v, wuv_v, bwo_v,
            x_v, gw_v, xs, qs, os_, qabs, macc, lacc, cacc, acca, accb, base,
            ksem, vsem, esem):
    def kcopy(i):
        return pltpu.make_async_copy(k_hbm.at[i], kbuf.at[i % 2], ksem)

    def vcopy(i, c):
        rows = pl.ds(VOFF[c], VSZ[c])
        return pltpu.make_async_copy(v_hbm.at[i, rows], vbuf.at[i % 2, rows], vsem.at[c])

    def ccopy(c):
        rows = pl.ds(c * CP, CP)
        return pltpu.make_async_copy(ckv_hbm.at[rows], ckv_v.at[rows], esem)

    wq_c = pltpu.make_async_copy(wq_hbm, wq_v, esem)
    x_c = pltpu.make_async_copy(x_hbm, x_v, esem)
    gw_c = pltpu.make_async_copy(gw_hbm, gw_v, esem)
    bwq_c = pltpu.make_async_copy(bwq_hbm, bwq_v, esem)
    wuk_c = pltpu.make_async_copy(wuk_hbm, wuk_v, esem)
    wuv_c = pltpu.make_async_copy(wuv_hbm, wuv_v, esem)
    bwo_c = pltpu.make_async_copy(bwo_hbm, bwo_v, esem)
    wo_c = pltpu.make_async_copy(wo_hbm.at[pl.ds(0, WOH)], wo_v.at[pl.ds(0, WOH)], esem)
    wo_t = pltpu.make_async_copy(wo_hbm.at[pl.ds(WOH, DH)], wo_v.at[pl.ds(WOH, DH)], esem)

    wq_c.start()
    x_c.start()
    gw_c.start()
    kcopy(0).start()
    for c in range(len(VSZ)):
        vcopy(0, c).start()

    row8 = jax.lax.broadcasted_iota(jnp.int32, (8, DH), 0)
    row16 = jax.lax.broadcasted_iota(jnp.int32, (16, DH), 0)

    xs[...] = jnp.zeros_like(xs)
    os_[...] = jnp.zeros_like(os_)
    acca[...] = jnp.zeros_like(acca)
    accb[...] = jnp.zeros_like(accb)
    base[...] = jnp.zeros_like(base)
    macc[...] = jnp.full(macc.shape, -jnp.inf, f32)
    lacc[...] = jnp.zeros_like(lacc)
    cacc[...] = jnp.zeros_like(cacc)

    x_c.wait()
    gw_c.wait()
    wq_c.wait()
    bwq_c.start()
    xs[0:B, :] = x_v[...].astype(f32)
    xb = xs[...].astype(bf16)

    def qproj(n, carry):
        cols = pl.ds(pl.multiple_of(n * 1024, 1024), 1024)
        qn = jnp.dot(xb, wq_v[:, cols], preferred_element_type=f32)
        for t in range(8):
            qs[n * 8 + t] = qn[:, t * DH:(t + 1) * DH]
        return carry

    jax.lax.fori_loop(0, 4, qproj, 0)

    bwq_u = bwq_v.bitcast(jnp.uint32)
    wuk_u = wuk_v.bitcast(jnp.uint32)
    wuv_u = wuv_v.bitcast(jnp.uint32)

    def step(i, carry):
        slot = i % 2
        b = i // H
        h = i % H

        q = qs[h].astype(bf16)
        kcopy(i).wait()

        @pl.when(i + 1 < NSTEP)
        def _():
            kcopy(i + 1).start()

        s = jax.lax.dot_general(q, kbuf[slot], NT, preferred_element_type=f32) * SCALE
        m = jnp.max(s, axis=1, keepdims=True)
        p = jnp.exp(s - m)
        l = jnp.sum(p, axis=1, keepdims=True)
        pb = p.astype(bf16)
        o = jnp.zeros((8, DH), f32)
        for c in range(len(VSZ)):
            vcopy(i, c).wait()

            @pl.when(i + 1 < NSTEP)
            def _():
                vcopy(i + 1, c).start()

            lo, hi = VOFF[c], VOFF[c] + VSZ[c]
            o = o + jnp.dot(pb[:, lo:hi], vbuf[slot, lo:hi, :], preferred_element_type=f32)

        @pl.when(i == NSTEP - 2)
        def _():
            wo_t.start()

        o = jnp.where(row8 == b, o / l, os_[h])

        @pl.when(b == 0)
        def _():
            os_[h] = o

        @pl.when((b == B - 1) & (i < NSTEP - 1))
        def _():
            w = wo_v[pl.ds(pl.multiple_of(h * DH, DH), DH), :]
            acca[...] += jnp.dot(o.astype(bf16), w, preferred_element_type=f32)

        @pl.when(i == NSTEP - 1)
        def _():
            gate = base[B:2 * B, :]
            pre = gate * acca[0:B, :] + base[0:B, :]
            ob = o.astype(bf16)
            wo_t.wait()
            last = jnp.dot(ob, wo_v[WOH:WOH + DH, :], preferred_element_type=f32)
            out_ref[...] = (gate * last[0:B, :] + pre).astype(out_ref.dtype)

        @pl.when(i <= S_BASE)
        def _():
            @pl.when(i == 0)
            def _():
                bwq_c.wait()
                wuk_c.start()

            @pl.when(i == 1)
            def _():
                wuk_c.wait()
                wuv_c.start()

            @pl.when(i == 2)
            def _():
                wuv_c.wait()
                bwo_c.start()

            @pl.when(i == 3)
            def _():
                bwo_c.wait()
                wo_c.start()

            @pl.when(i == 4)
            def _():
                wo_c.wait()
                ccopy(0).start()

            @pl.when((i >= S_BPROL) & (i < S_BPROL + 4))
            def _():
                g = i - S_BPROL
                xq = xs[...].astype(bf16)
                for r in range(4):
                    wq0, wq1 = _head_pair(bwq_u, g, r)
                    wk0, wk1 = _head_pair(wuk_u, g, r)
                    for t, (wqh, wkh) in enumerate(((wq0, wk0), (wq1, wk1))):
                        qh = jnp.dot(xq, wqh, preferred_element_type=f32).astype(bf16)
                        qa = jax.lax.dot_general(qh, wkh, NT, preferred_element_type=f32)
                        for bb in range(B):
                            qabs[pl.ds(bb * H + g * 8 + 2 * r + t, 1), :] = qa[bb:bb + 1, :]

            @pl.when((i >= S_CKV) & (i < S_CKV + NCP))
            def _():
                c = i - S_CKV
                ccopy(c).wait()

                @pl.when(c + 1 < NCP)
                def _():
                    ccopy(c + 1).start()

                bb = c // (SK // CP)
                qa = qabs[pl.ds(pl.multiple_of(bb * H, H), H), :].astype(bf16)

                def sub(u, carry2):
                    cc = ckv_v[pl.ds(pl.multiple_of(c * CP + u * CK, CK), CK), :]
                    sb = jax.lax.dot_general(qa, cc, NT, preferred_element_type=f32) * SCALE
                    m_old = macc[bb]
                    m_new = jnp.maximum(m_old, jnp.max(sb, axis=1, keepdims=True))
                    alpha = jnp.exp(m_old - m_new)
                    pp = jnp.exp(sb - m_new[:, 0:1])
                    lacc[bb] = alpha * lacc[bb] + jnp.sum(pp, axis=1, keepdims=True)
                    macc[bb] = m_new
                    pv = jnp.dot(pp.astype(bf16), cc, preferred_element_type=f32)
                    cacc[bb] = alpha[:, 0:1] * cacc[bb] + pv
                    return carry2

                jax.lax.fori_loop(0, CP // CK, sub, 0)

            @pl.when((i >= S_BEPI) & (i < S_BEPI + 4))
            def _():
                g = i - S_BEPI
                rows = pl.ds(pl.multiple_of(g * 8, 8), 8)
                lat = jnp.concatenate(
                    [cacc[bb, rows, :] / lacc[bb, rows, :][:, 0:1] for bb in range(B)],
                    axis=0).astype(bf16)
                acc = accb[...]
                for r in range(4):
                    for t, wv in enumerate(_head_pair(wuv_u, g, r)):
                        hr = 2 * r + t
                        ctx = jnp.dot(lat, wv, preferred_element_type=f32)
                        ctx = jnp.where((row16 % 8) == hr, ctx, 0.0).astype(bf16)
                        w = bwo_v[pl.ds(pl.multiple_of((g * 8 + hr) * DH, DH), DH), :]
                        acc = acc + jnp.dot(ctx, w, preferred_element_type=f32)
                accb[...] = acc

            @pl.when(i == S_BASE)
            def _():
                acc = accb[...]
                outb = jnp.concatenate(
                    [jnp.sum(acc[bb * 8:(bb + 1) * 8], axis=0, keepdims=True) for bb in range(B)],
                    axis=0)
                xf = x_v[...].astype(f32)
                z = jnp.sum(xf * gw_v[...].astype(f32).reshape(1, DM), axis=1, keepdims=True)
                gate = 1.0 / (1.0 + jnp.exp(-z))
                base[0:B, :] = (1.0 - gate) * outb
                base[B:2 * B, :] = jnp.broadcast_to(gate, (B, DM))

        return carry

    jax.lax.fori_loop(0, NSTEP, step, 0)


@jax.jit
def pallas_gated_mix__mha_block_cached__compressed_kv_cla__decode_kernel(
    A_x: jax.Array,
    A_k_cache: jax.Array,
    A_v_cache: jax.Array,
    A_wq: jax.Array,
    A_wo: jax.Array,
    B_x: jax.Array,
    B_c_kv: jax.Array,
    B_w_q: jax.Array,
    B_w_uk: jax.Array,
    B_w_uv: jax.Array,
    B_w_o: jax.Array,
    gate_w: jax.Array,
):
    del B_x
    hbm = pl.BlockSpec(memory_space=pl.ANY)
    out = pl.pallas_call(
        _kernel,
        out_shape=jax.ShapeDtypeStruct((B, DM), bf16),
        in_specs=[hbm] * 11,
        out_specs=pl.BlockSpec(memory_space=pltpu.VMEM),
        scratch_shapes=[
            pltpu.VMEM((2, SK, DH), bf16),
            pltpu.VMEM((2, SK, DH), bf16),
            pltpu.VMEM((DM, H * DH), bf16),
            pltpu.VMEM((H * DH, DM), bf16),
            pltpu.VMEM((B * SK, DC), bf16),
            pltpu.VMEM((DM * H, DH), bf16),
            pltpu.VMEM((DC * H, DH), bf16),
            pltpu.VMEM((DC * H, DH), bf16),
            pltpu.VMEM((H * DH, DM), bf16),
            pltpu.VMEM((B, DM), bf16),
            pltpu.VMEM((DM,), bf16),
            pltpu.VMEM((8, DM), f32),
            pltpu.VMEM((H, 8, DH), f32),
            pltpu.VMEM((H, 8, DH), f32),
            pltpu.VMEM((B * H, DC), f32),
            pltpu.VMEM((B, H, 128), f32),
            pltpu.VMEM((B, H, 128), f32),
            pltpu.VMEM((B, H, DC), f32),
            pltpu.VMEM((8, DM), f32),
            pltpu.VMEM((16, DM), f32),
            pltpu.VMEM((8, DM), f32),
            pltpu.SemaphoreType.DMA,
            pltpu.SemaphoreType.DMA((len(VSZ),)),
            pltpu.SemaphoreType.DMA,
        ],
        compiler_params=pltpu.CompilerParams(vmem_limit_bytes=96 * 2**20),
    )(
        A_x.reshape(B, DM), gate_w,
        A_k_cache.reshape(NSTEP, SK, DH), A_v_cache.reshape(NSTEP, SK, DH),
        A_wq, A_wo, B_c_kv.reshape(B * SK, DC),
        B_w_q.reshape(DM * H, DH), B_w_uk.reshape(DC * H, DH), B_w_uv.reshape(DC * H, DH),
        B_w_o.reshape(H * DH, DM),
    )
    return out.reshape(B, 1, DM)
```

```python
import jax
import jax.numpy as jnp
from jax.experimental import pallas as pl
from jax.experimental.pallas import tpu as pltpu

B, H, SK, DH, DM, DC = 2, 32, 8192, 128, 512, 512
NSTEP = B * H
CP = 2048
NCP = B * SK // CP
CK = 512
VSZ = (3072, 3072, 2048)
VOFF = (0, 3072, 6144)
WOH = (H - 1) * DH
SCALE = DH ** -0.5
NT = (((1,), (1,)), ((), ()))
f32 = jnp.float32
bf16 = jnp.bfloat16

S_BPROL = 2
S_CKV = 5
S_BEPI = S_CKV + NCP
S_BASE = S_BEPI + 4


def _stage_heads(w_ref, stage, g):
    w = w_ref[:, pl.ds(pl.multiple_of(g * 8, 8), 8), :]
    stage[...] = w.astype(f32).reshape(DM * 8, DH)


def _head(stage, r):
    return stage[pl.ds(r, DM, stride=8), :].astype(bf16)


def _kernel(x_hbm, gw_hbm, k_hbm, v_hbm, wq_hbm, wo_hbm, ckv_hbm, bwq_hbm, wuk_hbm,
            wuv_hbm, bwo_hbm, out_ref,
            kbuf, vbuf, wq_v, wo_v, ckv_v, bwq_v, wuk_v, wuv_v, bwo_v,
            x_v, gw_v, st0, st1, xs, qs, os_, qabs, macc, lacc, cacc, acca, accb, base,
            ksem, vsem, esem):
    def kcopy(i):
        return pltpu.make_async_copy(k_hbm.at[i], kbuf.at[i % 2], ksem)

    def vcopy(i, c):
        rows = pl.ds(VOFF[c], VSZ[c])
        return pltpu.make_async_copy(v_hbm.at[i, rows], vbuf.at[i % 2, rows], vsem.at[c])

    def ccopy(c):
        rows = pl.ds(c * CP, CP)
        return pltpu.make_async_copy(ckv_hbm.at[rows], ckv_v.at[rows], esem)

    wq_c = pltpu.make_async_copy(wq_hbm, wq_v, esem)
    x_c = pltpu.make_async_copy(x_hbm, x_v, esem)
    gw_c = pltpu.make_async_copy(gw_hbm, gw_v, esem)
    bwq_c = pltpu.make_async_copy(bwq_hbm, bwq_v, esem)
    wuk_c = pltpu.make_async_copy(wuk_hbm, wuk_v, esem)
    wuv_c = pltpu.make_async_copy(wuv_hbm, wuv_v, esem)
    bwo_c = pltpu.make_async_copy(bwo_hbm, bwo_v, esem)
    wo_c = pltpu.make_async_copy(wo_hbm.at[pl.ds(0, WOH)], wo_v.at[pl.ds(0, WOH)], esem)
    wo_t = pltpu.make_async_copy(wo_hbm.at[pl.ds(WOH, DH)], wo_v.at[pl.ds(WOH, DH)], esem)

    wq_c.start()
    x_c.start()
    gw_c.start()
    kcopy(0).start()
    for c in range(len(VSZ)):
        vcopy(0, c).start()

    row8 = jax.lax.broadcasted_iota(jnp.int32, (8, DH), 0)
    row16 = jax.lax.broadcasted_iota(jnp.int32, (16, DH), 0)

    xs[...] = jnp.zeros_like(xs)
    os_[...] = jnp.zeros_like(os_)
    acca[...] = jnp.zeros_like(acca)
    accb[...] = jnp.zeros_like(accb)
    base[...] = jnp.zeros_like(base)
    macc[...] = jnp.full(macc.shape, -jnp.inf, f32)
    lacc[...] = jnp.zeros_like(lacc)
    cacc[...] = jnp.zeros_like(cacc)

    x_c.wait()
    gw_c.wait()
    wq_c.wait()
    bwq_c.start()
    xs[0:B, :] = x_v[...].astype(f32)
    xb = xs[...].astype(bf16)

    def qproj(n, carry):
        cols = pl.ds(pl.multiple_of(n * 1024, 1024), 1024)
        qn = jnp.dot(xb, wq_v[:, cols], preferred_element_type=f32)
        for t in range(8):
            qs[n * 8 + t] = qn[:, t * DH:(t + 1) * DH]
        return carry

    jax.lax.fori_loop(0, 4, qproj, 0)

    def step(i, carry):
        slot = i % 2
        b = i // H
        h = i % H

        q = qs[h].astype(bf16)
        kcopy(i).wait()

        @pl.when(i + 1 < NSTEP)
        def _():
            kcopy(i + 1).start()

        s = jax.lax.dot_general(q, kbuf[slot], NT, preferred_element_type=f32) * SCALE
        m = jnp.max(s, axis=1, keepdims=True)
        p = jnp.exp(s - m)
        l = jnp.sum(p, axis=1, keepdims=True)
        pb = p.astype(bf16)
        o = jnp.zeros((8, DH), f32)
        for c in range(len(VSZ)):
            vcopy(i, c).wait()

            @pl.when(i + 1 < NSTEP)
            def _():
                vcopy(i + 1, c).start()

            lo, hi = VOFF[c], VOFF[c] + VSZ[c]
            o = o + jnp.dot(pb[:, lo:hi], vbuf[slot, lo:hi, :], preferred_element_type=f32)

        @pl.when(i == NSTEP - 2)
        def _():
            wo_t.start()

        o = jnp.where(row8 == b, o / l, os_[h])

        @pl.when(b == 0)
        def _():
            os_[h] = o

        @pl.when((b == B - 1) & (i < NSTEP - 1))
        def _():
            w = wo_v[pl.ds(pl.multiple_of(h * DH, DH), DH), :]
            acca[...] += jnp.dot(o.astype(bf16), w, preferred_element_type=f32)

        @pl.when(i == NSTEP - 1)
        def _():
            gate = base[B:2 * B, :]
            pre = gate * acca[0:B, :] + base[0:B, :]
            ob = o.astype(bf16)
            wo_t.wait()
            last = jnp.dot(ob, wo_v[WOH:WOH + DH, :], preferred_element_type=f32)
            out_ref[...] = (gate * last[0:B, :] + pre).astype(out_ref.dtype)

        @pl.when(i <= S_BASE)
        def _():
            @pl.when(i == 0)
            def _():
                bwq_c.wait()
                wuk_c.start()

            @pl.when(i == 1)
            def _():
                wuk_c.wait()
                wuv_c.start()

            @pl.when(i == 2)
            def _():
                wuv_c.wait()
                bwo_c.start()

            @pl.when(i == 3)
            def _():
                bwo_c.wait()
                wo_c.start()

            @pl.when(i == 4)
            def _():
                wo_c.wait()
                ccopy(0).start()

            @pl.when((i >= S_BPROL) & (i < S_BPROL + 4))
            def _():
                g = i - S_BPROL
                xq = xs[...].astype(bf16)
                _stage_heads(bwq_v, st0, g)
                _stage_heads(wuk_v, st1, g)
                for r in range(8):
                    qh = jnp.dot(xq, _head(st0, r), preferred_element_type=f32).astype(bf16)
                    qa = jax.lax.dot_general(qh, _head(st1, r), NT, preferred_element_type=f32)
                    for bb in range(B):
                        qabs[pl.ds(bb * H + g * 8 + r, 1), :] = qa[bb:bb + 1, :]

            @pl.when((i >= S_CKV) & (i < S_CKV + NCP))
            def _():
                c = i - S_CKV
                ccopy(c).wait()

                @pl.when(c + 1 < NCP)
                def _():
                    ccopy(c + 1).start()

                bb = c // (SK // CP)
                qa = qabs[pl.ds(pl.multiple_of(bb * H, H), H), :].astype(bf16)

                def sub(u, carry2):
                    cc = ckv_v[pl.ds(pl.multiple_of(c * CP + u * CK, CK), CK), :]
                    sb = jax.lax.dot_general(qa, cc, NT, preferred_element_type=f32) * SCALE
                    m_old = macc[bb]
                    m_new = jnp.maximum(m_old, jnp.max(sb, axis=1, keepdims=True))
                    alpha = jnp.exp(m_old - m_new)
                    pp = jnp.exp(sb - m_new[:, 0:1])
                    lacc[bb] = alpha * lacc[bb] + jnp.sum(pp, axis=1, keepdims=True)
                    macc[bb] = m_new
                    pv = jnp.dot(pp.astype(bf16), cc, preferred_element_type=f32)
                    cacc[bb] = alpha[:, 0:1] * cacc[bb] + pv
                    return carry2

                jax.lax.fori_loop(0, CP // CK, sub, 0)

            @pl.when((i >= S_BEPI) & (i < S_BEPI + 4))
            def _():
                g = i - S_BEPI
                rows = pl.ds(pl.multiple_of(g * 8, 8), 8)
                lat = jnp.concatenate(
                    [cacc[bb, rows, :] / lacc[bb, rows, :][:, 0:1] for bb in range(B)],
                    axis=0).astype(bf16)
                acc = accb[...]
                _stage_heads(wuv_v, st0, g)
                for r in range(8):
                    ctx = jnp.dot(lat, _head(st0, r), preferred_element_type=f32)
                    ctx = jnp.where((row16 % 8) == r, ctx, 0.0).astype(bf16)
                    w = bwo_v[pl.ds(pl.multiple_of((g * 8 + r) * DH, DH), DH), :]
                    acc = acc + jnp.dot(ctx, w, preferred_element_type=f32)
                accb[...] = acc

            @pl.when(i == S_BASE)
            def _():
                acc = accb[...]
                outb = jnp.concatenate(
                    [jnp.sum(acc[bb * 8:(bb + 1) * 8], axis=0, keepdims=True) for bb in range(B)],
                    axis=0)
                xf = x_v[...].astype(f32)
                z = jnp.sum(xf * gw_v[...].astype(f32).reshape(1, DM), axis=1, keepdims=True)
                gate = 1.0 / (1.0 + jnp.exp(-z))
                base[0:B, :] = (1.0 - gate) * outb
                base[B:2 * B, :] = jnp.broadcast_to(gate, (B, DM))

        return carry

    jax.lax.fori_loop(0, NSTEP, step, 0)


@jax.jit
def pallas_gated_mix__mha_block_cached__compressed_kv_cla__decode_kernel(
    A_x: jax.Array,
    A_k_cache: jax.Array,
    A_v_cache: jax.Array,
    A_wq: jax.Array,
    A_wo: jax.Array,
    B_x: jax.Array,
    B_c_kv: jax.Array,
    B_w_q: jax.Array,
    B_w_uk: jax.Array,
    B_w_uv: jax.Array,
    B_w_o: jax.Array,
    gate_w: jax.Array,
):
    del B_x
    hbm = pl.BlockSpec(memory_space=pl.ANY)
    out = pl.pallas_call(
        _kernel,
        out_shape=jax.ShapeDtypeStruct((B, DM), bf16),
        in_specs=[hbm] * 11,
        out_specs=pl.BlockSpec(memory_space=pltpu.VMEM),
        scratch_shapes=[
            pltpu.VMEM((2, SK, DH), bf16),
            pltpu.VMEM((2, SK, DH), bf16),
            pltpu.VMEM((DM, H * DH), bf16),
            pltpu.VMEM((H * DH, DM), bf16),
            pltpu.VMEM((B * SK, DC), bf16),
            pltpu.VMEM((DM, H, DH), bf16),
            pltpu.VMEM((DC, H, DH), bf16),
            pltpu.VMEM((DC, H, DH), bf16),
            pltpu.VMEM((H * DH, DM), bf16),
            pltpu.VMEM((B, DM), bf16),
            pltpu.VMEM((DM,), bf16),
            pltpu.VMEM((DM * 8, DH), f32),
            pltpu.VMEM((DM * 8, DH), f32),
            pltpu.VMEM((8, DM), f32),
            pltpu.VMEM((H, 8, DH), f32),
            pltpu.VMEM((H, 8, DH), f32),
            pltpu.VMEM((B * H, DC), f32),
            pltpu.VMEM((B, H, 128), f32),
            pltpu.VMEM((B, H, 128), f32),
            pltpu.VMEM((B, H, DC), f32),
            pltpu.VMEM((8, DM), f32),
            pltpu.VMEM((16, DM), f32),
            pltpu.VMEM((8, DM), f32),
            pltpu.SemaphoreType.DMA,
            pltpu.SemaphoreType.DMA((len(VSZ),)),
            pltpu.SemaphoreType.DMA,
        ],
        compiler_params=pltpu.CompilerParams(vmem_limit_bytes=96 * 2**20),
    )(
        A_x.reshape(B, DM), gate_w,
        A_k_cache.reshape(NSTEP, SK, DH), A_v_cache.reshape(NSTEP, SK, DH),
        A_wq, A_wo, B_c_kv.reshape(B * SK, DC),
        B_w_q, B_w_uk, B_w_uv,
        B_w_o.reshape(H * DH, DM),
    )
    return out.reshape(B, 1, DM)
```

```python
import jax
import jax.numpy as jnp
from jax.experimental import pallas as pl
from jax.experimental.pallas import tpu as pltpu

B, H, SK, DH, DM, DC = 2, 32, 8192, 128, 512, 512
NSTEP = B * H
CP = 2048
NCP = B * SK // CP
CK = 512
WOH = (H - 1) * DH
R, NS = 160, 4
PART = SK // NS
SCALE = DH ** -0.5
NT = (((1,), (1,)), ((), ()))
f32 = jnp.float32
bf16 = jnp.bfloat16

S_BPROL = 2
S_CKV = 5
S_BEPI = S_CKV + NCP
S_BASE = S_BEPI + 4


def _stage_heads(w_ref, stage, g):
    w = w_ref[:, pl.ds(pl.multiple_of(g * 8, 8), 8), :]
    stage[...] = w.astype(f32).reshape(DM * 8, DH)


def _head(stage, r):
    return stage[pl.ds(r, DM, stride=8), :].astype(bf16)


def _pieces(total, size):
    return [(o, min(size, total - o)) for o in range(0, total, size)]


def _kernel(x_hbm, gw_hbm, k_hbm, v_hbm, wq_hbm, wo_hbm, ckv_hbm, bwq_hbm, wuk_hbm,
            wuv_hbm, bwo_hbm, out_ref,
            kbuf, vbuf, wq_v, wo_v, ckv_v, bwq_v, wuk_v, wuv_v, bwo_v,
            x_v, gw_v, st0, st1, xs, qs, os_, qabs, macc, lacc, cacc, acca, accb, base,
            bsem):

    def sem_of(j):
        return bsem.at[(j + 1) % 3]

    def start_kv(j, do_k, do_v):
        sem = sem_of(j)
        kt, vt = j + 1, j
        for (o, r) in _pieces(PART, R):
            for n in range(NS):
                rows = pl.ds(n * PART + o, r)
                if do_k:
                    pltpu.make_async_copy(k_hbm.at[kt, rows], kbuf.at[kt % 3, rows], sem).start(priority=0)
                if do_v:
                    pltpu.make_async_copy(v_hbm.at[vt, rows], vbuf.at[vt % 3, rows], sem).start(priority=1)

    def wait_all(ref, j):
        pltpu.make_async_copy(ref, ref, sem_of(j)).wait()

    def start_rows(src, dst, j, lo=0, n=None):
        n = src.shape[0] if n is None else n
        pltpu.make_async_copy(src.at[pl.ds(lo, n)], dst.at[pl.ds(lo, n)], sem_of(j)).start(priority=0)

    def start_extra(j):
        if j == 0:
            start_rows(bwq_hbm, bwq_v, j)
        elif j == 1:
            start_rows(wuk_hbm, wuk_v, j)
        elif j == 2:
            start_rows(wuv_hbm, wuv_v, j)
        elif j == 3:
            start_rows(bwo_hbm, bwo_v, j)
        elif j == 4:
            start_rows(wo_hbm, wo_v, j)

    pltpu.make_async_copy(wq_hbm, wq_v, sem_of(-1)).start(priority=0)
    pltpu.make_async_copy(x_hbm, x_v, sem_of(-1)).start()
    pltpu.make_async_copy(gw_hbm, gw_v, sem_of(-1)).start()
    start_kv(-1, True, False)
    start_kv(0, True, True)
    start_extra(0)
    start_kv(1, True, True)
    start_extra(1)

    row8 = jax.lax.broadcasted_iota(jnp.int32, (8, DH), 0)
    row16 = jax.lax.broadcasted_iota(jnp.int32, (16, DH), 0)

    xs[...] = jnp.zeros_like(xs)
    os_[...] = jnp.zeros_like(os_)
    acca[...] = jnp.zeros_like(acca)
    accb[...] = jnp.zeros_like(accb)
    base[...] = jnp.zeros_like(base)
    macc[...] = jnp.full(macc.shape, -jnp.inf, f32)
    lacc[...] = jnp.zeros_like(lacc)
    cacc[...] = jnp.zeros_like(cacc)

    wait_all(wq_v, -1)
    wait_all(x_v, -1)
    wait_all(gw_v, -1)
    wait_all(kbuf.at[0], -1)
    xs[0:B, :] = x_v[...].astype(f32)
    xb = xs[...].astype(bf16)

    def qproj(n, carry):
        cols = pl.ds(pl.multiple_of(n * 1024, 1024), 1024)
        qn = jnp.dot(xb, wq_v[:, cols], preferred_element_type=f32)
        for t in range(8):
            qs[n * 8 + t] = qn[:, t * DH:(t + 1) * DH]
        return carry

    jax.lax.fori_loop(0, 4, qproj, 0)

    def step(i, carry):
        b = i // H
        h = i % H

        q = qs[h].astype(bf16)
        s = jax.lax.dot_general(q, kbuf[i % 3], NT, preferred_element_type=f32) * SCALE
        m = jnp.max(s, axis=1, keepdims=True)
        p = jnp.exp(s - m)
        l = jnp.sum(p, axis=1, keepdims=True)
        pb = p.astype(bf16)

        wait_all(vbuf.at[i % 3], i)

        @pl.when(i + 1 < NSTEP)
        def _():
            wait_all(kbuf.at[(i + 1) % 3], i)

        @pl.when(i <= S_CKV + NCP - 1)
        def _():
            for j, ref in ((0, bwq_v), (1, wuk_v), (2, wuv_v), (3, bwo_v), (4, wo_v)):
                @pl.when(i == j)
                def _():
                    wait_all(ref, j)

            @pl.when(i >= S_CKV)
            def _():
                wait_all(ckv_v.at[pl.ds(pl.multiple_of((i - S_CKV) * CP, CP), CP)], i)

        @pl.when(i + 3 < NSTEP)
        def _():
            start_kv(i + 2, True, True)

        @pl.when(i == NSTEP - 3)
        def _():
            start_kv(NSTEP - 1, False, True)

        @pl.when(i + 2 <= S_CKV + NCP - 1)
        def _():
            for j in (2, 3, 4):
                @pl.when(i + 2 == j)
                def _():
                    start_extra(j)

            @pl.when(i + 2 >= S_CKV)
            def _():
                start_rows(ckv_hbm, ckv_v, i + 2, lo=pl.multiple_of((i + 2 - S_CKV) * CP, CP), n=CP)

        o = jnp.dot(pb, vbuf[i % 3], preferred_element_type=f32)

        o = jnp.where(row8 == b, o / l, os_[h])

        @pl.when(b == 0)
        def _():
            os_[h] = o

        @pl.when((b == B - 1) & (i < NSTEP - 1))
        def _():
            w = wo_v[pl.ds(pl.multiple_of(h * DH, DH), DH), :]
            acca[...] += jnp.dot(o.astype(bf16), w, preferred_element_type=f32)

        @pl.when(i == NSTEP - 1)
        def _():
            gate = base[B:2 * B, :]
            pre = gate * acca[0:B, :] + base[0:B, :]
            ob = o.astype(bf16)
            last = jnp.dot(ob, wo_v[WOH:WOH + DH, :], preferred_element_type=f32)
            out_ref[...] = (gate * last[0:B, :] + pre).astype(out_ref.dtype)

        @pl.when(i <= S_BASE)
        def _():
            @pl.when((i >= S_BPROL) & (i < S_BPROL + 4))
            def _():
                g = i - S_BPROL
                xq = xs[...].astype(bf16)
                _stage_heads(bwq_v, st0, g)
                _stage_heads(wuk_v, st1, g)
                for r in range(8):
                    qh = jnp.dot(xq, _head(st0, r), preferred_element_type=f32).astype(bf16)
                    qa = jax.lax.dot_general(qh, _head(st1, r), NT, preferred_element_type=f32)
                    for bb in range(B):
                        qabs[pl.ds(bb * H + g * 8 + r, 1), :] = qa[bb:bb + 1, :]

            @pl.when((i >= S_CKV) & (i < S_CKV + NCP))
            def _():
                c = i - S_CKV
                bb = c // (SK // CP)
                qa = qabs[pl.ds(pl.multiple_of(bb * H, H), H), :].astype(bf16)

                def sub(u, carry2):
                    cc = ckv_v[pl.ds(pl.multiple_of(c * CP + u * CK, CK), CK), :]
                    sb = jax.lax.dot_general(qa, cc, NT, preferred_element_type=f32) * SCALE
                    m_old = macc[bb]
                    m_new = jnp.maximum(m_old, jnp.max(sb, axis=1, keepdims=True))
                    alpha = jnp.exp(m_old - m_new)
                    pp = jnp.exp(sb - m_new[:, 0:1])
                    lacc[bb] = alpha * lacc[bb] + jnp.sum(pp, axis=1, keepdims=True)
                    macc[bb] = m_new
                    pv = jnp.dot(pp.astype(bf16), cc, preferred_element_type=f32)
                    cacc[bb] = alpha[:, 0:1] * cacc[bb] + pv
                    return carry2

                jax.lax.fori_loop(0, CP // CK, sub, 0)

            @pl.when((i >= S_BEPI) & (i < S_BEPI + 4))
            def _():
                g = i - S_BEPI
                rows = pl.ds(pl.multiple_of(g * 8, 8), 8)
                lat = jnp.concatenate(
                    [cacc[bb, rows, :] / lacc[bb, rows, :][:, 0:1] for bb in range(B)],
                    axis=0).astype(bf16)
                acc = accb[...]
                _stage_heads(wuv_v, st0, g)
                for r in range(8):
                    ctx = jnp.dot(lat, _head(st0, r), preferred_element_type=f32)
                    ctx = jnp.where((row16 % 8) == r, ctx, 0.0).astype(bf16)
                    w = bwo_v[pl.ds(pl.multiple_of((g * 8 + r) * DH, DH), DH), :]
                    acc = acc + jnp.dot(ctx, w, preferred_element_type=f32)
                accb[...] = acc

            @pl.when(i == S_BASE)
            def _():
                acc = accb[...]
                outb = jnp.concatenate(
                    [jnp.sum(acc[bb * 8:(bb + 1) * 8], axis=0, keepdims=True) for bb in range(B)],
                    axis=0)
                xf = x_v[...].astype(f32)
                z = jnp.sum(xf * gw_v[...].astype(f32).reshape(1, DM), axis=1, keepdims=True)
                gate = 1.0 / (1.0 + jnp.exp(-z))
                base[0:B, :] = (1.0 - gate) * outb
                base[B:2 * B, :] = jnp.broadcast_to(gate, (B, DM))

        return carry

    jax.lax.fori_loop(0, NSTEP, step, 0)


@jax.jit
def pallas_gated_mix__mha_block_cached__compressed_kv_cla__decode_kernel(
    A_x: jax.Array,
    A_k_cache: jax.Array,
    A_v_cache: jax.Array,
    A_wq: jax.Array,
    A_wo: jax.Array,
    B_x: jax.Array,
    B_c_kv: jax.Array,
    B_w_q: jax.Array,
    B_w_uk: jax.Array,
    B_w_uv: jax.Array,
    B_w_o: jax.Array,
    gate_w: jax.Array,
):
    del B_x
    hbm = pl.BlockSpec(memory_space=pl.ANY)
    out = pl.pallas_call(
        _kernel,
        out_shape=jax.ShapeDtypeStruct((B, DM), bf16),
        in_specs=[hbm] * 11,
        out_specs=pl.BlockSpec(memory_space=pltpu.VMEM),
        scratch_shapes=[
            pltpu.VMEM((3, SK, DH), bf16),
            pltpu.VMEM((3, SK, DH), bf16),
            pltpu.VMEM((DM, H * DH), bf16),
            pltpu.VMEM((H * DH, DM), bf16),
            pltpu.VMEM((B * SK, DC), bf16),
            pltpu.VMEM((DM, H, DH), bf16),
            pltpu.VMEM((DC, H, DH), bf16),
            pltpu.VMEM((DC, H, DH), bf16),
            pltpu.VMEM((H * DH, DM), bf16),
            pltpu.VMEM((B, DM), bf16),
            pltpu.VMEM((DM,), bf16),
            pltpu.VMEM((DM * 8, DH), f32),
            pltpu.VMEM((DM * 8, DH), f32),
            pltpu.VMEM((8, DM), f32),
            pltpu.VMEM((H, 8, DH), f32),
            pltpu.VMEM((H, 8, DH), f32),
            pltpu.VMEM((B * H, DC), f32),
            pltpu.VMEM((B, H, 128), f32),
            pltpu.VMEM((B, H, 128), f32),
            pltpu.VMEM((B, H, DC), f32),
            pltpu.VMEM((8, DM), f32),
            pltpu.VMEM((16, DM), f32),
            pltpu.VMEM((8, DM), f32),
            pltpu.SemaphoreType.DMA((3,)),
        ],
        compiler_params=pltpu.CompilerParams(vmem_limit_bytes=96 * 2**20),
    )(
        A_x.reshape(B, DM), gate_w,
        A_k_cache.reshape(NSTEP, SK, DH), A_v_cache.reshape(NSTEP, SK, DH),
        A_wq, A_wo, B_c_kv.reshape(B * SK, DC),
        B_w_q, B_w_uk, B_w_uv,
        B_w_o.reshape(H * DH, DM),
    )
    return out.reshape(B, 1, DM)
```

```python
import jax
import jax.numpy as jnp
from jax.experimental import pallas as pl
from jax.experimental.pallas import tpu as pltpu

B, H, SK, DH, DM, DC = 2, 32, 8192, 128, 512, 512
NSTEP = B * H
SCALE = DH ** -0.5
NT = (((1,), (1,)), ((), ()))
f32 = jnp.float32
bf16 = jnp.bfloat16

NS = 4
R_KV = 160
R_3D = 6
R_2D = 56
VSZ = (3072, 3072, 2048)
VOFF = (0, 3072, 6144)
WOH = (H - 1) * DH
CP = 2048
NCP = B * SK // CP
CK = 512

S_BPROL = 2
S_CKV = 5
S_BEPI = S_CKV + NCP
S_BASE = S_BEPI + 4


def _pieces(total, size):
    return [(o, min(size, total - o)) for o in range(0, total, size)]


def _head_descriptors():
    part = SK // NS
    return [(n * part + o, r) for (o, r) in _pieces(part, R_KV) for n in range(NS)]


def _stage_heads(w_ref, stage, g):
    w = w_ref[:, pl.ds(pl.multiple_of(g * 8, 8), 8), :]
    stage[...] = w.astype(f32).reshape(DM * 8, DH)


def _head(stage, r):
    return stage[pl.ds(r, DM, stride=8), :].astype(bf16)


def _kernel(x_hbm, gw_hbm, k_hbm, v_hbm, wq_hbm, wo_hbm, ckv_hbm, bwq_hbm, wuk_hbm,
            wuv_hbm, bwo_hbm, out_ref,
            kbuf, vbuf, wq_v, wo_v, ckv_v, bwq_v, wuk_v, wuv_v, bwo_v, x_v, gw_v,
            pbuf, lbuf, st0, st1, xs, qs, os_, qabs, macc, lacc, cacc, acca, accb, base,
            bsem, tsem):
    descs = _head_descriptors()
    half_a, half_b = descs[:len(descs) // 2], descs[len(descs) // 2:]

    def sem_of(j):
        return bsem.at[(j + 1) % 3]

    def copy(src, dst, sem, queue):
        pltpu.make_async_copy(src, dst, sem).start(priority=queue)

    def start_kv(j, which):
        for (o, r) in which:
            rows = pl.ds(o, r)
            copy(k_hbm.at[j + 2, rows], kbuf.at[(j + 2) % 3, rows], sem_of(j), 0)
            copy(v_hbm.at[j, rows], vbuf.at[j % 3, rows], sem_of(j), 1)

    def start_halves(src, dst, sem, lo, n, rows_per_piece):
        half = n // 2
        for (o, r) in _pieces(half, rows_per_piece):
            for queue in range(2):
                rows = pl.ds(lo + queue * half + o, r)
                copy(src.at[rows], dst.at[rows], sem, queue)

    def start_weights(j):
        src, dst, n, rows = ((bwq_hbm, bwq_v, DM, R_3D), (wuk_hbm, wuk_v, DC, R_3D),
                             (wuv_hbm, wuv_v, DC, R_3D), (bwo_hbm, bwo_v, H * DH, R_2D),
                             (wo_hbm, wo_v, WOH, R_2D))[j]
        start_halves(src, dst, sem_of(j), 0, n, rows)

    def wait_all(ref, sem):
        pltpu.make_async_copy(ref, ref, sem).wait()

    wo_t = pltpu.make_async_copy(wo_hbm.at[pl.ds(WOH, DH)], wo_v.at[pl.ds(WOH, DH)],
                                 tsem.at[len(VSZ)])

    for r0 in range(0, DM // 2, 16):
        for (o, w) in _pieces(H * DH, 1536):
            for queue in range(2):
                idx = (pl.ds(queue * (DM // 2) + r0, 16), pl.ds(o, w))
                copy(wq_hbm.at[idx], wq_v.at[idx], sem_of(-1), queue)
    copy(x_hbm, x_v, sem_of(-1), 0)
    copy(gw_hbm, gw_v, sem_of(-1), 0)
    for (o, r) in descs:
        for t in range(2):
            copy(k_hbm.at[t, pl.ds(o, r)], kbuf.at[t, pl.ds(o, r)], sem_of(-1), t)
    start_kv(0, descs)
    start_weights(0)

    row8 = jax.lax.broadcasted_iota(jnp.int32, (8, DH), 0)
    row16 = jax.lax.broadcasted_iota(jnp.int32, (16, DH), 0)

    xs[...] = jnp.zeros_like(xs)
    os_[...] = jnp.zeros_like(os_)
    acca[...] = jnp.zeros_like(acca)
    accb[...] = jnp.zeros_like(accb)
    base[...] = jnp.zeros_like(base)
    macc[...] = jnp.full(macc.shape, -jnp.inf, f32)
    lacc[...] = jnp.zeros_like(lacc)
    cacc[...] = jnp.zeros_like(cacc)

    for ref in (wq_v, x_v, gw_v, kbuf.at[0], kbuf.at[1]):
        wait_all(ref, sem_of(-1))
    xs[0:B, :] = x_v[...].astype(f32)
    xb = xs[...].astype(bf16)

    def qproj(n, carry):
        cols = pl.ds(pl.multiple_of(n * 1024, 1024), 1024)
        qn = jnp.dot(xb, wq_v[:, cols], preferred_element_type=f32)
        for t in range(8):
            qs[n * 8 + t] = qn[:, t * DH:(t + 1) * DH]
        return carry

    jax.lax.fori_loop(0, 4, qproj, 0)

    def scores(t):
        q = qs[t % H].astype(bf16)
        s = jax.lax.dot_general(q, kbuf[t % 3], NT, preferred_element_type=f32) * SCALE
        m = jnp.max(s, axis=1, keepdims=True)
        p = jnp.exp(s - m)
        lbuf[t % 2] = jnp.broadcast_to(jnp.sum(p, axis=1, keepdims=True), (8, DH))
        pbuf[t % 2] = p.astype(bf16)

    scores(0)
    start_kv(1, descs)
    start_weights(1)

    def step(i, carry):
        b = i // H
        h = i % H

        scores(i + 1)

        wait_all(vbuf.at[i % 3], sem_of(i))

        @pl.when(i + 2 < NSTEP)
        def _():
            wait_all(kbuf.at[(i + 2) % 3], sem_of(i))

        @pl.when(i < S_CKV + NCP)
        def _():
            for j, ref in enumerate((bwq_v, wuk_v, wuv_v, bwo_v, wo_v.at[pl.ds(0, WOH)])):
                @pl.when(i == j)
                def _():
                    wait_all(ref, sem_of(j))

            @pl.when(i >= S_CKV)
            def _():
                wait_all(ckv_v.at[pl.ds(pl.multiple_of((i - S_CKV) * CP, CP), CP)], sem_of(i))

        @pl.when(i + 4 < NSTEP)
        def _():
            start_kv(i + 2, half_a)

        o = jnp.dot(pbuf[i % 2], vbuf[i % 3], preferred_element_type=f32)
        o = jnp.where(row8 == b, o / lbuf[i % 2], os_[h])

        @pl.when(b == 0)
        def _():
            os_[h] = o

        @pl.when(b == B - 1)
        def _():
            w = wo_v[pl.ds(pl.multiple_of(h * DH, DH), DH), :]
            acca[...] += jnp.dot(o.astype(bf16), w, preferred_element_type=f32)

        @pl.when(i + 2 < S_CKV + NCP)
        def _():
            for j in (2, 3, 4):
                @pl.when(i + 2 == j)
                def _():
                    start_weights(j)

            @pl.when(i + 2 >= S_CKV)
            def _():
                lo = pl.multiple_of((i + 2 - S_CKV) * CP, CP)
                start_halves(ckv_hbm, ckv_v, sem_of(i + 2), lo, CP, R_2D)

        @pl.when(i == NSTEP - 4)
        def _():
            t = NSTEP - 2
            start_halves(v_hbm.at[t], vbuf.at[t % 3], sem_of(t), 0, SK, R_KV)

        @pl.when(i == NSTEP - 3)
        def _():
            t = NSTEP - 1
            for c in range(len(VSZ)):
                start_halves(v_hbm.at[t], vbuf.at[t % 3], tsem.at[c], VOFF[c], VSZ[c], R_KV)
            wo_t.start()

        @pl.when(i <= S_BASE)
        def _():
            @pl.when((i >= S_BPROL) & (i < S_BPROL + 4))
            def _():
                g = i - S_BPROL
                xq = xs[...].astype(bf16)
                _stage_heads(bwq_v, st0, g)
                _stage_heads(wuk_v, st1, g)
                for r in range(8):
                    qh = jnp.dot(xq, _head(st0, r), preferred_element_type=f32).astype(bf16)
                    qa = jax.lax.dot_general(qh, _head(st1, r), NT, preferred_element_type=f32)
                    for bb in range(B):
                        qabs[pl.ds(bb * H + g * 8 + r, 1), :] = qa[bb:bb + 1, :]

            @pl.when((i >= S_CKV) & (i < S_CKV + NCP))
            def _():
                c = i - S_CKV
                bb = c // (SK // CP)
                qa = qabs[pl.ds(pl.multiple_of(bb * H, H), H), :].astype(bf16)

                def sub(u, carry2):
                    cc = ckv_v[pl.ds(pl.multiple_of(c * CP + u * CK, CK), CK), :]
                    sb = jax.lax.dot_general(qa, cc, NT, preferred_element_type=f32) * SCALE
                    m_old = macc[bb]
                    m_new = jnp.maximum(m_old, jnp.max(sb, axis=1, keepdims=True))
                    alpha = jnp.exp(m_old - m_new)
                    pp = jnp.exp(sb - m_new[:, 0:1])
                    lacc[bb] = alpha * lacc[bb] + jnp.sum(pp, axis=1, keepdims=True)
                    macc[bb] = m_new
                    pv = jnp.dot(pp.astype(bf16), cc, preferred_element_type=f32)
                    cacc[bb] = alpha[:, 0:1] * cacc[bb] + pv
                    return carry2

                jax.lax.fori_loop(0, CP // CK, sub, 0)

            @pl.when((i >= S_BEPI) & (i < S_BEPI + 4))
            def _():
                g = i - S_BEPI
                rows = pl.ds(pl.multiple_of(g * 8, 8), 8)
                lat = jnp.concatenate(
                    [cacc[bb, rows, :] / lacc[bb, rows, :][:, 0:1] for bb in range(B)],
                    axis=0).astype(bf16)
                acc = accb[...]
                _stage_heads(wuv_v, st0, g)
                for r in range(8):
                    ctx = jnp.dot(lat, _head(st0, r), preferred_element_type=f32)
                    ctx = jnp.where((row16 % 8) == r, ctx, 0.0).astype(bf16)
                    w = bwo_v[pl.ds(pl.multiple_of((g * 8 + r) * DH, DH), DH), :]
                    acc = acc + jnp.dot(ctx, w, preferred_element_type=f32)
                accb[...] = acc

            @pl.when(i == S_BASE)
            def _():
                acc = accb[...]
                outb = jnp.concatenate(
                    [jnp.sum(acc[bb * 8:(bb + 1) * 8], axis=0, keepdims=True) for bb in range(B)],
                    axis=0)
                xf = x_v[...].astype(f32)
                z = jnp.sum(xf * gw_v[...].astype(f32).reshape(1, DM), axis=1, keepdims=True)
                gate = 1.0 / (1.0 + jnp.exp(-z))
                base[0:B, :] = (1.0 - gate) * outb
                base[B:2 * B, :] = jnp.broadcast_to(gate, (B, DM))

        @pl.when(i + 4 < NSTEP)
        def _():
            start_kv(i + 2, half_b)

        return carry

    jax.lax.fori_loop(0, NSTEP - 1, step, 0)

    t = NSTEP - 1
    gate = base[B:2 * B, :]
    pre = gate * acca[0:B, :] + base[0:B, :]
    o = jnp.zeros((8, DH), f32)
    for c in range(len(VSZ)):
        chunk = vbuf.at[t % 3, pl.ds(VOFF[c], VSZ[c])]
        wait_all(chunk, tsem.at[c])
        o = o + jnp.dot(pbuf[t % 2, :, VOFF[c]:VOFF[c] + VSZ[c]], chunk[...],
                        preferred_element_type=f32)
    ob = jnp.where(row8 == B - 1, o / lbuf[t % 2], os_[H - 1]).astype(bf16)
    wo_t.wait()
    last = jnp.dot(ob, wo_v[WOH:WOH + DH, :], preferred_element_type=f32)
    out_ref[...] = (gate * last[0:B, :] + pre).astype(out_ref.dtype)


@jax.jit
def pallas_gated_mix__mha_block_cached__compressed_kv_cla__decode_kernel(
    A_x: jax.Array,
    A_k_cache: jax.Array,
    A_v_cache: jax.Array,
    A_wq: jax.Array,
    A_wo: jax.Array,
    B_x: jax.Array,
    B_c_kv: jax.Array,
    B_w_q: jax.Array,
    B_w_uk: jax.Array,
    B_w_uv: jax.Array,
    B_w_o: jax.Array,
    gate_w: jax.Array,
):
    del B_x
    hbm = pl.BlockSpec(memory_space=pl.ANY)
    out = pl.pallas_call(
        _kernel,
        out_shape=jax.ShapeDtypeStruct((B, DM), bf16),
        in_specs=[hbm] * 11,
        out_specs=pl.BlockSpec(memory_space=pltpu.VMEM),
        scratch_shapes=[
            pltpu.VMEM((3, SK, DH), bf16),
            pltpu.VMEM((3, SK, DH), bf16),
            pltpu.VMEM((DM, H * DH), bf16),
            pltpu.VMEM((H * DH, DM), bf16),
            pltpu.VMEM((B * SK, DC), bf16),
            pltpu.VMEM((DM, H, DH), bf16),
            pltpu.VMEM((DC, H, DH), bf16),
            pltpu.VMEM((DC, H, DH), bf16),
            pltpu.VMEM((H * DH, DM), bf16),
            pltpu.VMEM((B, DM), bf16),
            pltpu.VMEM((DM,), bf16),
            pltpu.VMEM((2, 8, SK), bf16),
            pltpu.VMEM((2, 8, DH), f32),
            pltpu.VMEM((DM * 8, DH), f32),
            pltpu.VMEM((DM * 8, DH), f32),
            pltpu.VMEM((8, DM), f32),
            pltpu.VMEM((H, 8, DH), f32),
            pltpu.VMEM((H, 8, DH), f32),
            pltpu.VMEM((B * H, DC), f32),
            pltpu.VMEM((B, H, 128), f32),
            pltpu.VMEM((B, H, 128), f32),
            pltpu.VMEM((B, H, DC), f32),
            pltpu.VMEM((8, DM), f32),
            pltpu.VMEM((16, DM), f32),
            pltpu.VMEM((8, DM), f32),
            pltpu.SemaphoreType.DMA((3,)),
            pltpu.SemaphoreType.DMA((len(VSZ) + 1,)),
        ],
        compiler_params=pltpu.CompilerParams(vmem_limit_bytes=96 * 2**20),
    )(
        A_x.reshape(B, DM), gate_w,
        A_k_cache.reshape(NSTEP, SK, DH), A_v_cache.reshape(NSTEP, SK, DH),
        A_wq, A_wo, B_c_kv.reshape(B * SK, DC),
        B_w_q, B_w_uk, B_w_uv,
        B_w_o.reshape(H * DH, DM),
    )
    return out.reshape(B, 1, DM)
```

```python
import jax
import jax.numpy as jnp
from jax.experimental import pallas as pl
from jax.experimental.pallas import tpu as pltpu

B, H, SK, DH, DM, DC = 2, 32, 8192, 128, 512, 512
NSTEP = B * H
SCALE = DH ** -0.5
NT = (((1,), (1,)), ((), ()))
f32 = jnp.float32
bf16 = jnp.bfloat16

NS = 4
R_KV = 160
R_3D = 6
R_2D = 56
R_WQ = 16
VSZ = (3072, 3072, 2048)
VOFF = (0, 3072, 6144)
WOH = (H - 1) * DH
CP = 2048
NCP = B * SK // CP
CK = 512

S_BPROL = 2
S_CKV = 5
S_BEPI = S_CKV + NCP
S_BASE = S_BEPI + 4


def _pieces(total, size):
    return [(o, min(size, total - o)) for o in range(0, total, size)]


def _head_descriptors():
    part = SK // NS
    return [(n * part + o, r) for (o, r) in _pieces(part, R_KV) for n in range(NS)]


def _stage_heads(w_ref, stage, g):
    w = w_ref[:, pl.ds(pl.multiple_of(g * 8, 8), 8), :]
    stage[...] = w.astype(f32).reshape(DM * 8, DH)


def _head(stage, r):
    return stage[pl.ds(r, DM, stride=8), :].astype(bf16)


def _kernel(x_hbm, gw_hbm, k_hbm, v_hbm, wq_hbm, wo_hbm, ckv_hbm, bwq_hbm, wuk_hbm,
            wuv_hbm, bwo_hbm, out_ref,
            kbuf, vbuf, wq_v, wo_v, ckv_v, bwq_v, wuk_v, wuv_v, bwo_v, x_v, gw_v,
            pbuf, lbuf, st0, st1, xs, qs, os_, qabs, macc, lacc, cacc, acca, accb, base,
            bsem, tsem):
    descs = _head_descriptors()
    half_a, half_b = descs[:len(descs) // 2], descs[len(descs) // 2:]

    def sem_of(j):
        return bsem.at[(j + 1) % 3]

    def copy(src, dst, sem, queue):
        pltpu.make_async_copy(src, dst, sem).start(priority=queue)

    def start_kv(j, which):
        for (o, r) in which:
            rows = pl.ds(o, r)
            copy(k_hbm.at[j + 2, rows], kbuf.at[(j + 2) % 3, rows], sem_of(j), 0)
            copy(v_hbm.at[j, rows], vbuf.at[j % 3, rows], sem_of(j), 1)

    def start_halves(src, dst, sem, lo, n, rows_per_piece):
        half = n // 2
        for (o, r) in _pieces(half, rows_per_piece):
            for queue in range(2):
                rows = pl.ds(lo + queue * half + o, r)
                copy(src.at[rows], dst.at[rows], sem, queue)

    def start_weights(j):
        src, dst, n, rows = ((bwq_hbm, bwq_v, DM, R_3D), (wuk_hbm, wuk_v, DC, R_3D),
                             (wuv_hbm, wuv_v, DC, R_3D), (bwo_hbm, bwo_v, H * DH, R_2D),
                             (wo_hbm, wo_v, WOH, R_2D))[j]
        start_halves(src, dst, sem_of(j), 0, n, rows)

    def wait_all(ref, sem):
        pltpu.make_async_copy(ref, ref, sem).wait()

    wo_t = pltpu.make_async_copy(wo_hbm.at[pl.ds(WOH, DH)], wo_v.at[pl.ds(WOH, DH)],
                                 tsem.at[len(VSZ)])

    start_halves(wq_hbm, wq_v, sem_of(-1), 0, DM, R_WQ)
    copy(x_hbm, x_v, sem_of(-1), 0)
    copy(gw_hbm, gw_v, sem_of(-1), 0)
    for (o, r) in descs:
        for t in range(2):
            copy(k_hbm.at[t, pl.ds(o, r)], kbuf.at[t, pl.ds(o, r)], sem_of(-1), t)
    start_kv(0, descs)
    start_weights(0)

    row8 = jax.lax.broadcasted_iota(jnp.int32, (8, DH), 0)
    row16 = jax.lax.broadcasted_iota(jnp.int32, (16, DH), 0)

    xs[...] = jnp.zeros_like(xs)
    os_[...] = jnp.zeros_like(os_)
    acca[...] = jnp.zeros_like(acca)
    accb[...] = jnp.zeros_like(accb)
    base[...] = jnp.zeros_like(base)
    macc[...] = jnp.full(macc.shape, -jnp.inf, f32)
    lacc[...] = jnp.zeros_like(lacc)
    cacc[...] = jnp.zeros_like(cacc)

    for ref in (wq_v, x_v, gw_v, kbuf.at[0], kbuf.at[1]):
        wait_all(ref, sem_of(-1))
    xs[0:B, :] = x_v[...].astype(f32)
    xb = xs[...].astype(bf16)

    def qproj(n, carry):
        cols = pl.ds(pl.multiple_of(n * 1024, 1024), 1024)
        qn = jnp.dot(xb, wq_v[:, cols], preferred_element_type=f32)
        for t in range(8):
            qs[n * 8 + t] = qn[:, t * DH:(t + 1) * DH]
        return carry

    jax.lax.fori_loop(0, 4, qproj, 0)

    def scores(t):
        q = qs[t % H].astype(bf16)
        s = jax.lax.dot_general(q, kbuf[t % 3], NT, preferred_element_type=f32) * SCALE
        m = jnp.max(s, axis=1, keepdims=True)
        p = jnp.exp(s - m)
        lbuf[t % 2] = jnp.broadcast_to(jnp.sum(p, axis=1, keepdims=True), (8, DH))
        pbuf[t % 2] = p.astype(bf16)

    scores(0)
    start_kv(1, descs)
    start_weights(1)

    def step(i, carry):
        b = i // H
        h = i % H

        scores(i + 1)

        wait_all(vbuf.at[i % 3], sem_of(i))

        @pl.when(i + 2 < NSTEP)
        def _():
            wait_all(kbuf.at[(i + 2) % 3], sem_of(i))

        @pl.when(i < S_CKV + NCP)
        def _():
            for j, ref in enumerate((bwq_v, wuk_v, wuv_v, bwo_v, wo_v.at[pl.ds(0, WOH)])):
                @pl.when(i == j)
                def _():
                    wait_all(ref, sem_of(j))

            @pl.when(i >= S_CKV)
            def _():
                wait_all(ckv_v.at[pl.ds(pl.multiple_of((i - S_CKV) * CP, CP), CP)], sem_of(i))

        @pl.when(i + 4 < NSTEP)
        def _():
            start_kv(i + 2, half_a)

        o = jnp.dot(pbuf[i % 2], vbuf[i % 3], preferred_element_type=f32)
        o = jnp.where(row8 == b, o / lbuf[i % 2], os_[h])

        @pl.when(b == 0)
        def _():
            os_[h] = o

        @pl.when(b == B - 1)
        def _():
            w = wo_v[pl.ds(pl.multiple_of(h * DH, DH), DH), :]
            acca[...] += jnp.dot(o.astype(bf16), w, preferred_element_type=f32)

        @pl.when(i + 2 < S_CKV + NCP)
        def _():
            for j in (2, 3, 4):
                @pl.when(i + 2 == j)
                def _():
                    start_weights(j)

            @pl.when(i + 2 >= S_CKV)
            def _():
                lo = pl.multiple_of((i + 2 - S_CKV) * CP, CP)
                start_halves(ckv_hbm, ckv_v, sem_of(i + 2), lo, CP, R_2D)

        @pl.when(i == NSTEP - 4)
        def _():
            t = NSTEP - 2
            start_halves(v_hbm.at[t], vbuf.at[t % 3], sem_of(t), 0, SK, R_KV)

        @pl.when(i == NSTEP - 3)
        def _():
            t = NSTEP - 1
            for c in range(len(VSZ)):
                start_halves(v_hbm.at[t], vbuf.at[t % 3], tsem.at[c], VOFF[c], VSZ[c], R_KV)
            wo_t.start()

        @pl.when(i <= S_BASE)
        def _():
            @pl.when((i >= S_BPROL) & (i < S_BPROL + 4))
            def _():
                g = i - S_BPROL
                xq = xs[...].astype(bf16)
                _stage_heads(bwq_v, st0, g)
                _stage_heads(wuk_v, st1, g)
                for r in range(8):
                    qh = jnp.dot(xq, _head(st0, r), preferred_element_type=f32).astype(bf16)
                    qa = jax.lax.dot_general(qh, _head(st1, r), NT, preferred_element_type=f32)
                    for bb in range(B):
                        qabs[pl.ds(bb * H + g * 8 + r, 1), :] = qa[bb:bb + 1, :]

            @pl.when((i >= S_CKV) & (i < S_CKV + NCP))
            def _():
                c = i - S_CKV
                bb = c // (SK // CP)
                qa = qabs[pl.ds(pl.multiple_of(bb * H, H), H), :].astype(bf16)

                def sub(u, carry2):
                    cc = ckv_v[pl.ds(pl.multiple_of(c * CP + u * CK, CK), CK), :]
                    sb = jax.lax.dot_general(qa, cc, NT, preferred_element_type=f32) * SCALE
                    m_old = macc[bb]
                    m_new = jnp.maximum(m_old, jnp.max(sb, axis=1, keepdims=True))
                    alpha = jnp.exp(m_old - m_new)
                    pp = jnp.exp(sb - m_new[:, 0:1])
                    lacc[bb] = alpha * lacc[bb] + jnp.sum(pp, axis=1, keepdims=True)
                    macc[bb] = m_new
                    pv = jnp.dot(pp.astype(bf16), cc, preferred_element_type=f32)
                    cacc[bb] = alpha[:, 0:1] * cacc[bb] + pv
                    return carry2

                jax.lax.fori_loop(0, CP // CK, sub, 0)

            @pl.when((i >= S_BEPI) & (i < S_BEPI + 4))
            def _():
                g = i - S_BEPI
                rows = pl.ds(pl.multiple_of(g * 8, 8), 8)
                lat = jnp.concatenate(
                    [cacc[bb, rows, :] / lacc[bb, rows, :][:, 0:1] for bb in range(B)],
                    axis=0).astype(bf16)
                acc = accb[...]
                _stage_heads(wuv_v, st0, g)
                for r in range(8):
                    ctx = jnp.dot(lat, _head(st0, r), preferred_element_type=f32)
                    ctx = jnp.where((row16 % 8) == r, ctx, 0.0).astype(bf16)
                    w = bwo_v[pl.ds(pl.multiple_of((g * 8 + r) * DH, DH), DH), :]
                    acc = acc + jnp.dot(ctx, w, preferred_element_type=f32)
                accb[...] = acc

            @pl.when(i == S_BASE)
            def _():
                acc = accb[...]
                outb = jnp.concatenate(
                    [jnp.sum(acc[bb * 8:(bb + 1) * 8], axis=0, keepdims=True) for bb in range(B)],
                    axis=0)
                xf = x_v[...].astype(f32)
                z = jnp.sum(xf * gw_v[...].astype(f32).reshape(1, DM), axis=1, keepdims=True)
                gate = 1.0 / (1.0 + jnp.exp(-z))
                base[0:B, :] = (1.0 - gate) * outb
                base[B:2 * B, :] = jnp.broadcast_to(gate, (B, DM))

        @pl.when(i + 4 < NSTEP)
        def _():
            start_kv(i + 2, half_b)

        return carry

    jax.lax.fori_loop(0, NSTEP - 1, step, 0)

    t = NSTEP - 1
    gate = base[B:2 * B, :]
    pre = gate * acca[0:B, :] + base[0:B, :]
    o = jnp.zeros((8, DH), f32)
    for c in range(len(VSZ)):
        chunk = vbuf.at[t % 3, pl.ds(VOFF[c], VSZ[c])]
        wait_all(chunk, tsem.at[c])
        o = o + jnp.dot(pbuf[t % 2, :, VOFF[c]:VOFF[c] + VSZ[c]], chunk[...],
                        preferred_element_type=f32)
    ob = jnp.where(row8 == B - 1, o / lbuf[t % 2], os_[H - 1]).astype(bf16)
    wo_t.wait()
    last = jnp.dot(ob, wo_v[WOH:WOH + DH, :], preferred_element_type=f32)
    out_ref[...] = (gate * last[0:B, :] + pre).astype(out_ref.dtype)


@jax.jit
def pallas_gated_mix__mha_block_cached__compressed_kv_cla__decode_kernel(
    A_x: jax.Array,
    A_k_cache: jax.Array,
    A_v_cache: jax.Array,
    A_wq: jax.Array,
    A_wo: jax.Array,
    B_x: jax.Array,
    B_c_kv: jax.Array,
    B_w_q: jax.Array,
    B_w_uk: jax.Array,
    B_w_uv: jax.Array,
    B_w_o: jax.Array,
    gate_w: jax.Array,
):
    del B_x
    hbm = pl.BlockSpec(memory_space=pl.ANY)
    out = pl.pallas_call(
        _kernel,
        out_shape=jax.ShapeDtypeStruct((B, DM), bf16),
        in_specs=[hbm] * 11,
        out_specs=pl.BlockSpec(memory_space=pltpu.VMEM),
        scratch_shapes=[
            pltpu.VMEM((3, SK, DH), bf16),
            pltpu.VMEM((3, SK, DH), bf16),
            pltpu.VMEM((DM, H * DH), bf16),
            pltpu.VMEM((H * DH, DM), bf16),
            pltpu.VMEM((B * SK, DC), bf16),
            pltpu.VMEM((DM, H, DH), bf16),
            pltpu.VMEM((DC, H, DH), bf16),
            pltpu.VMEM((DC, H, DH), bf16),
            pltpu.VMEM((H * DH, DM), bf16),
            pltpu.VMEM((B, DM), bf16),
            pltpu.VMEM((DM,), bf16),
            pltpu.VMEM((2, 8, SK), bf16),
            pltpu.VMEM((2, 8, DH), f32),
            pltpu.VMEM((DM * 8, DH), f32),
            pltpu.VMEM((DM * 8, DH), f32),
            pltpu.VMEM((8, DM), f32),
            pltpu.VMEM((H, 8, DH), f32),
            pltpu.VMEM((H, 8, DH), f32),
            pltpu.VMEM((B * H, DC), f32),
            pltpu.VMEM((B, H, 128), f32),
            pltpu.VMEM((B, H, 128), f32),
            pltpu.VMEM((B, H, DC), f32),
            pltpu.VMEM((8, DM), f32),
            pltpu.VMEM((16, DM), f32),
            pltpu.VMEM((8, DM), f32),
            pltpu.SemaphoreType.DMA((3,)),
            pltpu.SemaphoreType.DMA((len(VSZ) + 1,)),
        ],
        compiler_params=pltpu.CompilerParams(vmem_limit_bytes=96 * 2**20),
    )(
        A_x.reshape(B, DM), gate_w,
        A_k_cache.reshape(NSTEP, SK, DH), A_v_cache.reshape(NSTEP, SK, DH),
        A_wq, A_wo, B_c_kv.reshape(B * SK, DC),
        B_w_q, B_w_uk, B_w_uv,
        B_w_o.reshape(H * DH, DM),
    )
    return out.reshape(B, 1, DM)
```
